```python
import os as _os
_os.environ.setdefault('JAX_PLATFORMS', 'cpu')
import jax
import jax.numpy as jnp

def _softmax(x, axis=-1):
    return jax.nn.softmax(x, axis=axis)

def _gelu(x):
    return jax.nn.gelu(x, approximate=True)

def _silu(x):
    return jax.nn.silu(x)

def _sigmoid(x):
    return jax.nn.sigmoid(x)

def _layernorm(x, axis=-1, eps=1e-05):
    m = jnp.mean(x, axis=axis, keepdims=True)
    v = jnp.var(x, axis=axis, keepdims=True)
    return (x - m) / jnp.sqrt(v + eps)

def _scatter_add(tgt, idx, src, axis=0):
    return tgt.at[idx].add(src)

def _segment_sum(src, seg, n):
    return jax.ops.segment_sum(src, seg, n)

class _Rng:

    def __init__(self, key):
        self._k = key

    def _next(self):
        self._k, sub = jax.random.split(self._k)
        return sub

    def normal(self, shape):
        return jax.random.normal(self._next(), shape, dtype=jnp.bfloat16)

    def randint(self, lo, hi, shape):
        return jax.random.randint(self._next(), shape, lo, hi, dtype=jnp.int32)

    def uniform(self, shape, lo=0.0, hi=1.0):
        return jax.random.uniform(self._next(), shape, jnp.bfloat16, lo, hi)

    def permutation(self, n):
        return jax.random.permutation(self._next(), n)
kernel_name = 'adaLN_cond__mha_block__geglu_ffn__prompt'

def setup_inputs():
    _rng = _Rng(jax.random.key(int.from_bytes(__import__("os").urandom(4), "little")))
    _w = lambda a: (lambda t: t.astype(jnp.bfloat16) if jnp.issubdtype(t.dtype, jnp.floating) else t)(jnp.asarray(a))

    def _A_setup():
        B, S, D, H = (1, 2048, 512, 32)
        return {'x': _w((lambda *s: _rng.normal(s) * 0.05)(B, S, D)), 'wqkv': _w((lambda *s: _rng.normal(s) * 0.05)(D, 3 * D)), 'wo': _w((lambda *s: _rng.normal(s) * 0.05)(D, D))}
    _A_in = _A_setup()

    def _B_setup():
        B, S, D, F = (1, 2048, 512, 1376)
        return {'x': _w((lambda *s: _rng.normal(s) * 0.05)(B, S, D)), 'w_gate': _w((lambda *s: _rng.normal(s) * 0.05)(D, F)), 'w_up': _w((lambda *s: _rng.normal(s) * 0.05)(D, F)), 'w_down': _w((lambda *s: _rng.normal(s) * 0.05)(F, D))}
    _B_in = _B_setup()
    return {'A_x': _A_in['x'], 'A_wqkv': _A_in['wqkv'], 'A_wo': _A_in['wo'], 'B_x': _B_in['x'], 'B_w_gate': _B_in['w_gate'], 'B_w_up': _B_in['w_up'], 'B_w_down': _B_in['w_down'], 'c': _w((lambda *s: _rng.normal(s) * 0.05)(1, 512) * 8.0), 'w_mod': _w((lambda *s: _rng.normal(s) * 0.05)(512, 6 * 512) * 512 ** (-0.5) * 8.0)}

def reference(A_x, A_wqkv, A_wo, B_x, B_w_gate, B_w_up, B_w_down, c, w_mod):

    def _A_ref(x, wqkv, wo):
        B, S, D = x.shape
        H = 32
        Dh = D // H
        qkv = (lambda x, *d: x.transpose(*d))((x @ wqkv).reshape(B, S, 3, H, Dh), 2, 0, 3, 1, 4)
        q, k, v = (qkv[0], qkv[1], qkv[2])
        scores = jnp.einsum('bhqd,bhkd->bhqk', q, k) * Dh ** (-0.5)
        p = _softmax(scores, axis=-1)
        o = jnp.einsum('bhqk,bhkd->bhqd', p, v)
        return (lambda x, *d: x.transpose(*d))(o, 0, 2, 1, 3).reshape(B, S, D) @ wo

    def _B_ref(x, w_gate, w_up, w_down):
        return _gelu(x @ w_gate) * (x @ w_up) @ w_down
    x = A_x
    mod = (_silu(c) @ w_mod).reshape(c.shape[0], 6, 1, -1)
    sa, ca, ga, sb, cb, gb = (mod[:, 0].copy(), mod[:, 1].copy(), mod[:, 2].copy(), mod[:, 3].copy(), mod[:, 4].copy(), mod[:, 5].copy())
    h = _layernorm(x, axis=-1) * (1 + ca) + sa
    x = x + ga * _A_ref(h, A_wqkv, A_wo)
    h = _layernorm(x, axis=-1) * (1 + cb) + sb
    x = x + gb * _B_ref(h, B_w_gate, B_w_up, B_w_down)
    return x
```

```python
import functools
import math

import jax
import jax.numpy as jnp
from jax import lax
import jax.experimental.pallas as pl
import jax.experimental.pallas.tpu as pltpu


S, D, H, DH, F = 2048, 512, 32, 16, 1376
LANES = 128
NT = S // LANES
HPG = LANES // DH
EPS = 1e-5
Q_SCALE = DH ** -0.5 * math.log2(math.e)

TM1 = 512
TM3 = 512
NV = 16
APOS = 7
NL = 2

BF16, F32, U32 = jnp.bfloat16, jnp.float32, jnp.uint32


def _as_bf16(x):
    return pltpu.bitcast(x, BF16)


def _pack(x):
    return pltpu.bitcast(x.astype(BF16), U32)


def _dot(a, b):
    return jnp.dot(a, b, preferred_element_type=F32)


def _dot_t(a, b):
    return lax.dot_general(a, b, (((1,), (1,)), ((), ())), preferred_element_type=F32)


def _layernorm(x):
    xc = x - jnp.mean(x, axis=-1, keepdims=True)
    var = jnp.mean(xc * xc, axis=-1, keepdims=True)
    return xc * lax.rsqrt(var + EPS)


def _gelu(x):
    c = math.sqrt(2.0 / math.pi)
    hx = 0.5 * x
    return hx + hx * jnp.tanh(x * (c + (c * 0.044715) * (x * x)))


GROUPS = 8
NTILE = NT * NT
RING = 16
LAG = RING - 4
VPOS = [int(v) for v in "4,0".split(",")]
XTRA = [int(v) for v in "-1".split(",")]
XMOD = 16
NVT = 2 if XTRA != [-1] else 1


TB = 8


def _tile(n):
    b, w = divmod(n, TB * NT)
    return b * TB + w % TB, w // TB


def _vpu_rows(n):
    return VPOS[:2] if n % XMOD in XTRA else VPOS[:1]


def _mxu_rows(n):
    return [r for r in range(GROUPS - 1, -1, -1) if r not in _vpu_rows(n)]


LEAD = [int(v) for v in "2,3,5,7".split(",")]


def _mxu_program():
    ops = []
    for j in range(4):
        rows = _mxu_rows(LAG + j)
        cut = max(len(rows) - LEAD[j], 0)
        lane = [("qk", LAG + j, rows[cut:])]
        for n in range(j, NTILE, 4):
            m = n + LAG + 4
            lane += [("pv", n, None), ("qk", m, _mxu_rows(m) if n + 4 < NTILE else rows[:cut])]
        ops.append([op for op in lane if op[0] == "pv" or op[2]])
    order, load, ptr = [], [0] * 4, [0] * 4
    while any(ptr[j] < len(ops[j]) for j in range(4)):
        j = min((j for j in range(4) if ptr[j] < len(ops[j])), key=lambda j: (load[j], j))
        op = ops[j][ptr[j]]
        ptr[j] += 1
        load[j] += max(2, 1 if op[0] == "pv" else len(op[2]))
        order.append(op)
    if 0:
        for j in range(4):
            print(j, " ".join("P" if o[0] == "pv" else str(len(o[2])) for o in ops[j][:30]))
        print(load)
    return order


def _kernel(c_ref, x_hbm, wqkv_hbm, wo_hbm, wg_hbm, wu_hbm, wd_hbm, wm_hbm, out_hbm,
            x_v, wqkv_v, wo_v, wg_v, wu_v, wd_v, wm_v, mod_v,
            k_all, k_f32, q_t, v_t, k_lhs, k_bc, s_buf, l_acc, o_acc, o_t, out_v, sems, out_sems):
    n1 = S // TM1

    def x_copy(i):
        rows = pl.ds(i * TM1, TM1)
        return pltpu.make_async_copy(x_hbm.at[rows], x_v.at[rows], sems.at[8 + i])

    wm_a = pltpu.make_async_copy(wm_hbm.at[:, pl.ds(0, 2 * D)], wm_v.at[:, pl.ds(0, 2 * D)], sems.at[0])
    wm_b = pltpu.make_async_copy(wm_hbm.at[:, pl.ds(2 * D, 4 * D)], wm_v.at[:, pl.ds(2 * D, 4 * D)], sems.at[1])
    w_qkv = pltpu.make_async_copy(wqkv_hbm, wqkv_v, sems.at[2])
    late = [wm_b] + [
        pltpu.make_async_copy(src, dst, sems.at[3 + i])
        for i, (src, dst) in enumerate(((wo_hbm, wo_v), (wg_hbm, wg_v), (wu_hbm, wu_v), (wd_hbm, wd_v)))
    ]

    wm_a.start()
    x_copy(0).start()
    w_qkv.start()
    for i in range(1, n1):
        x_copy(i).start()

    c = c_ref[...].astype(F32)
    sc = jnp.broadcast_to(c * jax.nn.sigmoid(c), (16, D)).astype(BF16)
    wm_a.wait()
    mod_v[:, 0:2 * D] = _dot(sc, wm_v[:, 0:2 * D])[0:8]
    w_qkv.wait()
    for cp in late:
        cp.start()

    def mod(i):
        return mod_v[0:1, i * D:(i + 1) * D]

    for i in range(n1):
        x_copy(i).wait()
        x = x_v[pl.ds(i * TM1, TM1), :].astype(F32)
        hb = (_layernorm(x) * (1.0 + mod(1)) + mod(0)).astype(BF16)
        cols = pl.ds(i * TM1, TM1)
        k = _dot(hb, wqkv_v[:, D:2 * D])
        for g in range(D // LANES):
            kg = k[:, g * LANES:(g + 1) * LANES]
            k_all[g, pl.ds(i * TM1 // 2, TM1 // 2), :] = _pack(kg)
            for t in range(TM1 // LANES):
                for n in range(NVT):
                    r0 = t * LANES + 16 * VPOS[n]
                    k_f32[g, pl.ds(((i * TM1 // LANES + t) * NVT + n) * 16, 16), :] = kg[r0:r0 + 16]
        q_t[:, cols] = (_dot(hb, wqkv_v[:, 0:D]) * Q_SCALE).T
        v_t[:, cols] = _pack(_dot(hb, wqkv_v[:, 2 * D:3 * D]).T)

    def head_rows(h, n):
        return pl.ds(pl.multiple_of(h * n, n), n)

    def q_rhs(h, u):
        q = q_t[head_rows(h, DH), u * LANES:(u + 1) * LANES]
        return jnp.concatenate([q, jnp.zeros((LANES - DH, LANES), F32)], axis=0).astype(BF16)

    def head_of(i):
        return (i // HPG) * HPG + (HPG - 1 - i % HPG)

    def stage_mxu_keys(i, b):
        rows = pl.ds(b * TB * LANES // 2, TB * LANES // 2)
        k = pltpu.roll(k_all[i % H // HPG, rows, :], DH, 1)
        k_lhs[b % 2][0] = k
        k_all[i // HPG, rows, :] = k

    def stage_vpu_keys(i, b):
        sel = pl.ds(b * TB * NVT * 16, TB * NVT * 16)
        k = pltpu.roll(k_f32[i % H // HPG, sel, :], DH, 1)
        k_f32[i // HPG, sel, :] = k
        nb = 2 * 16
        for r0 in range(0, TB * NVT * 16, nb):
            for d in range(DH):
                k_bc[b % 2][0, d, pl.ds(r0, nb), :] = jnp.broadcast_to(k[r0:r0 + nb, d:d + 1], (nb, LANES))

    def scores(h, m, rows, zero):
        t, u = _tile(m)
        r0 = (t % TB) * LANES // 2
        lhs = jnp.concatenate([k_lhs[t // TB % 2][zero, pl.ds(r0 + 8 * r, 8), :] for r in rows], axis=0)
        s = _dot(_as_bf16(lhs), q_rhs(h, u))
        for n, r in enumerate(rows):
            s_buf[m % RING, pl.ds(16 * r, 16), :] = s[16 * n:16 * n + 16]

    stage_mxu_keys(0, 0)
    stage_vpu_keys(0, 0)
    for m in range(RING):
        scores(head_of(0), m, _mxu_rows(m), 0)

    program = _mxu_program()
    n_blk = NT // TB

    def head_body(i, carry):
        lo, hi = carry
        nxt = i + 1
        h, hn = head_of(i), head_of(nxt % H)
        qv = q_t.at[head_rows(h, DH)]
        vv = v_t.at[head_rows(h, DH // 2)]
        mxu_staged = vpu_staged = 0
        l_run, o_run = {}, {}
        zero = [lax.shift_right_logical(i + u, 10) if 0 else 0 for u in range(NTILE // TB + 4)]
        for kind, n, rows in program:
            t, u = _tile(n)
            b = t // TB
            if kind == "qk":
                if b > mxu_staged:
                    mxu_staged = b
                    stage_mxu_keys(*((i, b) if b < n_blk else (nxt, 0)))
                scores(h if b < n_blk else hn, n % NTILE, rows, zero[n // TB])
                continue
            if b >= vpu_staged and u >= NT // 2:
                vpu_staged = b + 1
                stage_vpu_keys(*((i, b + 1) if b + 1 < n_blk else (nxt, 0)))
            cols = slice(u * LANES, (u + 1) * LANES)
            p, lt = {}, None
            for r in range(GROUPS - 1, -1, -1):
                if r in _vpu_rows(n):
                    r0 = ((t % TB) * NVT + VPOS.index(r)) * 16
                    s = None
                    for d in range(DH):
                        term = k_bc[b % 2][zero[n // TB], d, pl.ds(r0, 16), :] * qv[d:d + 1, cols]
                        s = term if s is None else s + term
                else:
                    s = s_buf[n % RING, pl.ds(16 * r, 16), :]
                p[r] = jnp.exp2(s)
                pair = p[r][0:8] + p[r][8:16]
                lt = pair if lt is None else lt + pair
            pt = jnp.concatenate([p[r] for r in range(GROUPS)], axis=0).astype(BF16)
            ot = _dot(_as_bf16(vv[:, t * LANES:(t + 1) * LANES]), pt)
            cnt, lp, op = l_run.get((b, u), (0, None, None))
            lt, ot = (lt, ot) if cnt == 0 else (lp + lt, op + ot)
            l_run[b, u] = (cnt + 1, lt, ot)
            if cnt + 1 < TB:
                continue
            if b > 0:
                lt = lt + l_acc[:, cols]
                ot = ot + o_acc[:, cols]
            if b < n_blk - 1:
                l_acc[:, cols] = lt
                o_acc[:, cols] = ot
            else:
                lsum = jnp.sum(lt, axis=0, keepdims=True)
                o_t[head_rows(h, DH), cols] = ot * (1.0 / lsum)
                lo = jnp.minimum(lo, lsum)
                hi = jnp.maximum(hi, lsum)
        return lo, hi

    one = jnp.ones((1, LANES), F32)
    lo, hi = lax.fori_loop(0, H, head_body, (one, one))
    safe = jnp.logical_and(jnp.min(lo) >= 2.0 ** -30, jnp.max(hi) <= 2.0 ** 40)

    @pl.when(jnp.logical_not(safe))
    def _():
        def body(i, _):
            h, u = i // NT, i % NT
            cols = pl.ds(pl.multiple_of(u * LANES, LANES), LANES)
            grp_rows = pl.ds(pl.multiple_of((h // HPG) * LANES, LANES), LANES)
            row_head = lax.broadcasted_iota(jnp.int32, (LANES, LANES), 0) // DH
            q = jnp.where(row_head == h % HPG, q_t[grp_rows, cols], 0.0).astype(BF16)
            s = _dot(_as_bf16(k_all[h // HPG]), q)
            p = jnp.exp2(s - jnp.max(s, axis=0, keepdims=True))
            ot = _dot(_as_bf16(v_t[head_rows(h, DH // 2), :]), p.astype(BF16))
            o_t[head_rows(h, DH), cols] = ot / jnp.sum(p, axis=0, keepdims=True)

        lax.fori_loop(0, H * NT, body, None)

    for cp in late:
        cp.wait()
    mod_v[:, 2 * D:6 * D] = _dot(sc, wm_v[:, 2 * D:6 * D])[0:8]

    def out_copy(i):
        rows = pl.ds(pl.multiple_of(i * TM3, TM3), TM3)
        return pltpu.make_async_copy(out_v.at[rows], out_hbm.at[rows], out_sems.at[i])

    def ffn_body(i, _):
        rows = pl.ds(pl.multiple_of(i * TM3, TM3), TM3)
        attn = _dot(o_t[:, rows].T.astype(BF16), wo_v[...])
        x1 = x_v[rows, :].astype(F32) + mod(2) * attn
        hb = (_layernorm(x1) * (1.0 + mod(4)) + mod(3)).astype(BF16)
        a = (_gelu(_dot_t(hb, wg_v[...])) * _dot_t(hb, wu_v[...])).astype(BF16)
        out_v[rows, :] = (x1 + mod(5) * _dot(a, wd_v[...])).astype(out_v.dtype)
        out_copy(i).start()

    lax.fori_loop(0, S // TM3, ffn_body, None)
    for i in range(S // TM3):
        out_copy(i).wait()


@jax.jit
def pallas_adaLN_cond__mha_block__geglu_ffn__prompt_kernel(
    A_x, A_wqkv, A_wo, B_x, B_w_gate, B_w_up, B_w_down, c, w_mod
):
    del B_x
    hbm = pl.BlockSpec(memory_space=pltpu.HBM)
    out = pl.pallas_call(
        _kernel,
        name="blk",
        out_shape=jax.ShapeDtypeStruct((S, D), A_x.dtype),
        in_specs=[pl.BlockSpec(memory_space=pltpu.VMEM)] + [hbm] * 7,
        out_specs=hbm,
        scratch_shapes=[
            pltpu.VMEM((S, D), BF16),
            pltpu.VMEM((D, 3 * D), BF16),
            pltpu.VMEM((D, D), BF16),
            pltpu.VMEM((F, D), BF16),
            pltpu.VMEM((F, D), BF16),
            pltpu.VMEM((F, D), BF16),
            pltpu.VMEM((D, 6 * D), BF16),
            pltpu.VMEM((8, 6 * D), F32),
            pltpu.VMEM((D // LANES + 1, S // 2, LANES), U32),
            pltpu.VMEM((D // LANES + 1, NT * NVT * 16, LANES), F32),
            pltpu.VMEM((D, S), F32),
            pltpu.VMEM((D // 2, S), U32),
            [pltpu.VMEM((2, TB * LANES // 2, LANES), U32)] * 2,
            [pltpu.VMEM((2, DH, TB * NVT * 16, LANES), F32)] * 2,
            pltpu.VMEM((RING, LANES, LANES), F32),
            pltpu.VMEM((8, S), F32),
            pltpu.VMEM((DH, S), F32),
            pltpu.VMEM((D, S), F32),
            pltpu.VMEM((S, D), BF16),
            pltpu.SemaphoreType.DMA((8 + S // TM1,)),
            pltpu.SemaphoreType.DMA((S // TM3,)),
        ],
        compiler_params=pltpu.CompilerParams(vmem_limit_bytes=100 * 2**20),
    )(c, A_x.reshape(S, D), A_wqkv, A_wo, B_w_gate.T, B_w_up.T, B_w_down, w_mod)
    return out.reshape(A_x.shape)
```

```python
import functools
import math

import jax
import jax.numpy as jnp
from jax import lax
import jax.experimental.pallas as pl
import jax.experimental.pallas.tpu as pltpu


S, D, H, DH, F = 2048, 512, 32, 16, 1376
LANES, SUB, N_MXU = 128, 8, 4
NT = S // LANES
HPG = LANES // DH
EPS = 1e-5
F32_MAX = 3.4028234663852886e38
Q_SCALE = DH ** -0.5 * math.log2(math.e)

BF16, F32, U32 = jnp.bfloat16, jnp.float32, jnp.uint32

TM = 512
HM, HD = TM // 2, D // 2
NR = 16

G = LANES // SUB
TB = 8
N_BLK = NT // TB
HEAD_STEPS = N_BLK * NT
NH = 2
VPU_ROWS = [(t, r) for t in range(TB) for r in ((2, 6) if t % 2 else (2, 6, 12))]
MXU_ROWS = [(t, r) for t in range(TB) for r in reversed(range(G)) if (t, r) not in VPU_ROWS]
N_MM = len(MXU_ROWS) // 2
AHEAD = 45
Q_HELD = 12

SUM_MIN, SUM_MAX, V_MAX = 2.0 ** -60, 2.0 ** 90, 2.0 ** 30

LEFT = ((0, 3, 1), (2, 3, 1), (0, None, 0), (3, None, 0), (0, 1, 1), (2, 0, -1), (1, 3, -1))
RIGHT = ((0, 3, 1), (0, None, 0), (1, 3, -1), (2, 0, -1), (3, None, 0), (0, 1, 1), (2, 3, 1))
USES = (((0, 1), (3, 1)), ((2, 1), (3, -1)), ((1, 1), (3, 1)), ((0, 1), (2, 1)),
        ((0, -1), (1, 1)), ((3, 1),), ((0, 1),))


def _pack(x):
    return pltpu.bitcast(x.astype(BF16), U32)


def _unpack(x):
    return pltpu.bitcast(x, BF16)


def _dot(a, b):
    return lax.dot_general(a, b, (((1,), (0,)), ((), ())), preferred_element_type=F32)


def _dot_t(a, b):
    return lax.dot_general(a, b, (((1,), (1,)), ((), ())), preferred_element_type=F32)


def _layernorm(x):
    xc = x - jnp.mean(x, axis=-1, keepdims=True)
    var = jnp.mean(xc * xc, axis=-1, keepdims=True)
    return xc * lax.rsqrt(var + EPS)


def _gelu(x):
    c = math.sqrt(2.0 / math.pi)
    hx = 0.5 * x
    return hx + hx * jnp.tanh(x * (c + (c * 0.044715) * (x * x)))


def _factor(spec, block):
    first, second, sign = spec
    x = block(*divmod(first, 2))
    if second is None:
        return x
    x, y = x.astype(F32), block(*divmod(second, 2)).astype(F32)
    return x + y if sign > 0 else x - y


def _accumulate(out, n, product):
    for quadrant, sign in USES[n]:
        if quadrant in out:
            out[quadrant] = out[quadrant] + product if sign > 0 else out[quadrant] - product
        else:
            out[quadrant] = product if sign > 0 else -product


def _after(x, zeros):
    if zeros is None:
        return x
    head = [x[0:SUB, 0:LANES] + zeros] + [x[0:SUB, LANES:]] * (x.shape[1] > LANES)
    return jnp.concatenate([jnp.concatenate(head, axis=1), x[SUB:]], axis=0)


def _block(i, n):
    return pl.ds(i * n if isinstance(i, int) else pl.multiple_of(i * n, n), n)


def _runs(values):
    runs = []
    for v in values:
        if runs and sum(runs[-1]) == v:
            runs[-1][1] += 1
        else:
            runs.append([v, 1])
    return runs


def _attention_program():
    n_tile = NH * HEAD_STEPS * TB
    n_slot = NH * HEAD_STEPS * (N_MM + TB) // N_MXU
    grid = [[None] * n_slot for _ in range(N_MXU)]
    for n in range(n_tile):
        grid[n % N_MXU][min((5 * n + 6) * n_slot // (5 * n_tile), n_slot - 1)] = ("pv", n, [None])
    free = [(j, slot) for slot in range(n_slot) for j in range(N_MXU) if grid[j][slot] is None]
    step_at = {at: (i + AHEAD) // N_MM for i, at in enumerate(free)}

    def alone(j, slot):
        return step_at.get((j, slot - 1)) != step_at[j, slot] != step_at.get((j, slot + 1))

    for i, at in enumerate(free):
        for other in sorted(free[max(i - 8, 0):i + 9], key=lambda o: abs(o[1] - at[1])):
            if alone(*at) and step_at[other] != step_at[at]:
                step_at[at], step_at[other] = step_at[other], step_at[at]
                near = [(j, slot + k) for j, slot in (at, other) for k in (-1, 0, 1)]
                if any(alone(*o) for o in near if o in step_at):
                    step_at[at], step_at[other] = step_at[other], step_at[at]
    taken = {0: AHEAD}
    for j, slot in free:
        step = step_at[j, slot]
        grid[j][slot] = ("qk", step, [taken.get(step, 0)])
        taken[step] = taken.get(step, 0) + 1

    queues = []
    for row in grid:
        queue = []
        for op in row:
            if op[0] == "qk" and queue and queue[-1][:2] == op[:2]:
                queue[-1][2].extend(op[2])
            else:
                queue.append(op)
        queues.append(queue)
    program, load = [], [0] * N_MXU
    while any(queues):
        j = min((j for j in range(N_MXU) if queues[j]), key=lambda j: (load[j], j))
        program.append(queues[j].pop(0))
        load[j] += max(2, len(program[-1][2]))
    return program


def _attention_scratch():
    vmem, groups = pltpu.VMEM, D // LANES
    return [
        vmem((D, S), F32),
        vmem((D // 2, S), U32),
        vmem((groups, S // 2, LANES), U32),
        vmem((groups, N_BLK * N_MM * SUB, LANES), U32),
        vmem((D // 2, S), U32),
        vmem((D, S), F32),
        vmem((groups, N_BLK * len(VPU_ROWS) * SUB, LANES), F32),
        vmem(((2 * HPG - 1) * SUB, S), U32),
        [vmem((2, len(VPU_ROWS), DH, SUB, LANES), F32)] * N_BLK,
        vmem((2 * AHEAD * SUB, LANES), F32),
        vmem((DH + SUB, S), F32),
    ]


def _attention(v_peak, q_t, q_pk, k_pk, k_mxu, v_pk, o_t, k_vpu, q_win, k_bc, s_buf, acc):
    def stage_keys(h, b):
        keys = k_vpu[h >> 3, _block(b, len(VPU_ROWS) * SUB), :]
        for d in range(DH):
            lane = jnp.full(keys.shape, (h & (HPG - 1)) * DH + d, jnp.int32)
            column = jnp.take_along_axis(keys, lane, axis=1, mode="promise_in_bounds")
            k_bc[b][0, :, d] = column.reshape(len(VPU_ROWS), SUB, LANES)

    def stage_queries(h, cols):
        q_win[_block(HPG - 1, SUB), cols] = q_pk[_block(h, SUB), cols]

    def mxu_scores(h, step, passes):
        b, u = divmod(step % HEAD_STEPS, NT)
        keys = [k_mxu[h >> 3, pl.ds((b * N_MM + r) * SUB, n * SUB), :] for r, n in _runs(passes)]
        window = pl.ds(pl.multiple_of((HPG - 1 - (h & (HPG - 1))) * SUB, SUB), HPG * SUB)
        return _dot(_unpack(jnp.concatenate(keys, axis=0)), _unpack(q_win[window, _block(u, LANES)]))

    stage_keys(0, 0)
    stage_queries(0, slice(None))
    part = pl.cdiv(AHEAD, N_MXU)
    first = [mxu_scores(0, 0, range(k * part, (k + 1) * part)) for k in range(N_MXU)]
    s_buf[...] = jnp.concatenate(first, axis=0)[:s_buf.shape[0]]
    program = _attention_program()

    def body(i, bad):
        heads = [(i * NH + e) & (H - 1) for e in range(NH + 1)]
        ready, queries, running = {}, {}, {}
        for kind, n, passes in program:
            if kind == "qk":
                s = mxu_scores(heads[n // HEAD_STEPS], n, passes)
                for k, mm in enumerate(passes):
                    if n == NH * HEAD_STEPS:
                        s_buf[_block(mm, 2 * SUB), :] = s[2 * SUB * k:2 * SUB * (k + 1)]
                    else:
                        for g in range(2):
                            ready[n, MXU_ROWS[2 * mm + g]] = s[SUB * (2 * k + g):SUB * (2 * k + g + 1)]
                continue

            step, t = divmod(n, TB)
            (b, u), h = divmod(step % HEAD_STEPS, NT), heads[step // HEAD_STEPS]
            cols = _block(u, LANES)
            if step not in queries:
                q_rows = q_t.at[_block(h, DH)]
                q_all = q_rows[:, cols]
                q = [q_all[d:d + 1] if d < Q_HELD else q_rows[d:d + 1, cols] for d in range(DH)]
                queries[step] = (lax.shift_right_logical(i + step, 10),
                                 jnp.stack([jnp.broadcast_to(row, (SUB, LANES)) for row in q]))
                if u == 1:
                    assert step == 1 or running[step - 2][0] == TB
                    stage_keys(heads[(step // NT + 1) // N_BLK], (b + 1) % N_BLK)
                if b == N_BLK - 1 and u > 0:
                    assert all((step - 1, row) in ready for row in MXU_ROWS)
                    stage_queries(heads[step // HEAD_STEPS + 1], _block(u - 1, LANES))
                if b == 0 and u == 1:
                    stage_queries(h, _block(NT - 1, LANES))

            zero, q = queries[step]
            rows = []
            for r in range(G):
                if (t, r) in VPU_ROWS:
                    terms = k_bc[b][zero, VPU_ROWS.index((t, r))] * q
                    rows.append(jnp.sum(jnp.sum(terms.reshape(DH // 4, 4, SUB, LANES), axis=0), axis=0))
                elif step == 0 and MXU_ROWS.index((t, r)) < 2 * AHEAD:
                    rows.append(s_buf[_block(MXU_ROWS.index((t, r)), SUB), :])
                else:
                    rows.append(ready[step, (t, r)])
            p = jnp.exp2(jnp.concatenate(rows, axis=0))
            o = _dot(_unpack(v_pk[_block(h, SUB), _block(b * TB + t, LANES)]), p)
            total = functools.reduce(jnp.add, [p[r * SUB:(r + 1) * SUB] for r in reversed(range(G))])

            count, total_prev, o_prev = running.get(step, (0, None, None))
            if count:
                total, o = total_prev + total, o + o_prev
            running[step] = (count + 1, total, o)
            if count + 1 < TB:
                continue
            if b > 0:
                total, o = total + acc[DH:, cols], o + acc[0:DH, cols]
            if b < N_BLK - 1:
                acc[DH:, cols], acc[0:DH, cols] = total, o
            else:
                total = jnp.sum(total, axis=0, keepdims=True)
                o_t[_block(h, DH), cols] = o * (1.0 / total)
                bad = jnp.where((total >= SUM_MIN) & (total <= SUM_MAX), bad, 1.0)
        return bad

    bad = jnp.where(jnp.max(v_peak, axis=0, keepdims=True) <= V_MAX, 0.0, 1.0)
    bad = lax.fori_loop(0, H // NH, body, bad)

    @pl.when(jnp.max(bad) > 0.0)
    def _():
        def exact(i, _):
            h, cols = i // (S // TM), _block(i % (S // TM), TM)
            row_head = lax.broadcasted_iota(jnp.int32, (LANES, TM), 0) // DH
            q = jnp.where(row_head == h % HPG, q_t[_block(h // HPG, LANES), cols], 0.0).astype(BF16)

            def tile(t, carry):
                m_old, total, o = carry
                s = _dot(_unpack(k_pk[h // HPG, _block(t, LANES // 2), :]), q)
                m = jnp.maximum(m_old, jnp.max(s, axis=0, keepdims=True))
                p, keep = jnp.exp2(s - m), jnp.exp2(m_old - m)
                v = _unpack(v_pk[_block(h, SUB), _block(t, LANES)])
                return m, keep * total + jnp.sum(p, axis=0, keepdims=True), keep * o + _dot(v, p)

            start = jnp.full((1, TM), -F32_MAX, F32), jnp.zeros((1, TM), F32), jnp.zeros((DH, TM), F32)
            _, total, o = lax.fori_loop(0, NT, tile, start)
            o_t[_block(h, DH), cols] = o / total

        lax.fori_loop(0, H * (S // TM), exact, None)


def _kernel(c_hbm, x_hbm, wqkv_hbm, wo_hbm, wg_hbm, wu_hbm, wd_hbm, wm_hbm, out_hbm,
            c_v, x_v, wqkv_v, wo_v, wg_v, wu_v, wd_v, wm_v, mod_v, attn_refs,
            h_v, h_terms, wo_terms, a_terms, x1_v, out_v, sems, out_sem):
    q_t, q_pk, k_pk, k_mxu, v_pk, o_t, k_vpu, q_win = attn_refs[:8]

    def x_rows(r0, n):
        return x_hbm.at[pl.ds(r0, n)], x_v.at[pl.ds(r0, n)]

    def wm_cols(c0, n):
        return wm_hbm.at[:, pl.ds(c0, n)], wm_v.at[:, pl.ds(c0, n)]

    def qkv_part(p):
        return wqkv_hbm.at[:, pl.ds(p * D, D)], wqkv_v.at[:, pl.ds(p * D, D)]

    copies = [
        pltpu.make_async_copy(src, dst, sems.at[n])
        for n, (src, dst) in enumerate((
            (c_hbm, c_v), x_rows(0, TM), wm_cols(0, 2 * D), qkv_part(1),
            qkv_part(0), x_rows(TM, TM),
            qkv_part(2), x_rows(2 * TM, S - 2 * TM),
            wm_cols(2 * D, 4 * D), (wo_hbm, wo_v), (wg_hbm, wg_v), (wu_hbm, wu_v), (wd_hbm, wd_v),
        ))
    ]
    for cp in copies:
        cp.start()
    (c_copy, x_head, wm_head, wk), second, third, late = copies[0:4], copies[4:6], copies[6:8], copies[8:]

    zero = lax.fori_loop(0, 2, lambda i, z: z - i, 1)
    h_v[0:SUB, 0:LANES] = jnp.zeros((SUB, LANES), F32)
    q_win[...] = jnp.zeros(q_win.shape, U32)

    def mod(i):
        return mod_v[0:1, i * D:(i + 1) * D]

    def token_rows(i, half, r0, n):
        return _block(i * (TM // n) + (half * HM + r0) // n, n)

    def h_rows(half, r0, n):
        return pl.ds(SUB + half * HM + r0, n)

    def make_terms(slot, halves=None):
        halves = halves or [h_v[h_rows(half, 0, HM), :] for half in range(2)]
        for n in range(7):
            h_terms[slot, n] = _factor(LEFT[n], lambda r, c: halves[r][:, c * HD:(c + 1) * HD])

    issued = []

    def spread(steps, n_dots, source=None, lag=4):
        calls, started, pending = 0, 0, []

        def tick(can_wait=True):
            nonlocal calls, started
            calls += 1
            due = min(-(-calls * len(steps) // (n_dots - lag)), len(steps))
            if started < due:
                if issued:
                    spare = pl.ds(pl.multiple_of(S - 16 * zero, 16), 16)
                    source[spare, 0:LANES] = issued[-1][0:16, 0:LANES].astype(source.dtype)
                pending.extend((calls, step()) for step in steps[started:due])
                started = due
            zeros = None
            if can_wait and pending and pending[0][0] + lag <= calls:
                while pending and pending[0][0] + lag <= calls:
                    rows, value = pending.pop(0)[1]
                    h_v[rows] = value
                zeros = h_v[_block(zero, SUB), 0:LANES]
            assert calls < n_dots or not pending
            return zeros

        return tick

    idle = spread([], 14)

    def strassen(dot, slot, w, tick):
        out = {}
        for n in (0, 1, 5, 2, 4, 3, 6):
            issued.append(dot(h_terms[slot, n], _after(_factor(RIGHT[n], w), tick(RIGHT[n][1] is not None))))
            _accumulate(out, n, issued[-1])
        return [out[k] for k in range(4)]

    def norm_steps(i):
        def step(half, r0):
            x = x_v[token_rows(i, half, r0, NR), :].astype(F32)
            return h_rows(half, r0, NR), _layernorm(x) * (1.0 + mod(1)) + mod(0)

        return [functools.partial(step, half, r0) for r0 in range(0, HM, NR) for half in range(2)]

    v_peaks = []

    def project(i, part, tick):
        for j in range(2):
            def w(r, c):
                return wqkv_v[_block(r, HD), pl.ds(part * D + (j + 2 * c) * LANES, LANES)]

            quadrants = strassen(_dot, i % 2, w, tick)
            for c in range(2):
                g, y = j + 2 * c, jnp.concatenate(quadrants[c::2], axis=0)
                if part == 0:
                    yt = (y * Q_SCALE).T
                    q_t[_block(g, LANES), _block(i, TM)] = yt
                    q_pk[_block(g, LANES // 2), _block(i, TM)] = _pack(yt)
                elif part == 2:
                    v_pk[_block(g, LANES // 2), _block(i, TM)] = _pack(y.T)
                    v_peaks.append(jnp.max(jnp.abs(y).reshape(TM // SUB, SUB, LANES), axis=0))
                else:
                    k_pk[g, _block(i, TM // 2), :] = _pack(y)
                    for groups, dst, convert in ((MXU_ROWS, k_mxu, _pack), (VPU_ROWS, k_vpu, lambda k: k)):
                        starts = [t * LANES + r * SUB for t, r in groups if t * LANES < TM]
                        keys = convert(jnp.concatenate([y[r0:r0 + SUB] for r0 in starts], axis=0))
                        dst[g, _block(i, keys.shape[0]), :] = keys

    c_copy.wait()
    cond = c_v[...].astype(F32)
    cond = jnp.broadcast_to(cond * jax.nn.sigmoid(cond), (SUB, D))
    x_head.wait()
    x1_v[0:TM, :] = _layernorm(x_v[0:TM, :].astype(F32))
    wm_head.wait()
    mod_v[:, 0:2 * D] = _dot(cond, wm_v[:, 0:2 * D])
    make_terms(0, [x1_v[_block(half, HM), :] * (1.0 + mod(1)) + mod(0) for half in range(2)])
    wk.wait()
    project(0, 1, idle)
    for cp in second:
        cp.wait()
    project(0, 0, spread(norm_steps(1), 14, x_v))
    make_terms(1)
    project(1, 1, idle)
    for cp in third:
        cp.wait()
    tick = spread(norm_steps(2), 42, x_v)
    for i, part in ((0, 2), (1, 0), (1, 2)):
        project(i, part, tick)
    make_terms(0)
    tick = spread(norm_steps(3), 42, x_v)
    for part in (1, 0, 2):
        project(2, part, tick)
    make_terms(1)
    for part in (0, 2, 1):
        project(3, part, idle)

    _attention(functools.reduce(jnp.maximum, v_peaks), *attn_refs)

    for cp in late:
        cp.wait()
    n_chunk, n_ft = S // TM, pl.cdiv(F, LANES)
    n_pair = n_ft // 2

    def norm2_steps(i):
        def step(half, r0):
            if r0 % LANES == 0:
                rows = token_rows(i, half, r0, LANES)
                x1_v[rows, :] = x_v[rows, :].astype(F32) + mod(2) * o_t[:, rows].T
            x = x1_v[token_rows(i, half, r0, NR), :]
            return h_rows(half, r0, NR), _layernorm(x) * (1.0 + mod(4)) + mod(3)

        return [functools.partial(step, half, r0) for half in range(2) for r0 in range(0, HM, NR)]

    wo_t = {(r, c): wo_v[_block(r, HD), _block(c, HD)].T for r in range(2) for c in range(2)}
    for n in range(7):
        wo_terms[n] = _factor(RIGHT[n], lambda r, c: wo_t[r, c]).astype(BF16)
    issued.clear()
    tick = spread(norm2_steps(0), 14, x1_v, lag=3)
    for i in range(n_chunk):
        def quadrant(half, c):
            return _block(c, HD), token_rows(i, half, 0, HM)

        out = {}
        for n in (1, 5, 3, 6, 4, 0, 2):
            heads = _factor(LEFT[n], lambda half, c: o_t[quadrant(half, c)])
            issued.append(_dot(wo_terms[n], _after(heads, tick() if i >= n_chunk - 2 else None)))
            _accumulate(out, n, issued[-1])
            if len(issued) <= 4 * D // LANES:
                cols = pl.ds(2 * D + (len(issued) - 1) * LANES, LANES)
                mod_v[:, cols] = _dot(cond, wm_v[:, cols])
        for k, y in out.items():
            o_t[quadrant(*divmod(k, 2))] = y

    def ffn(i, _):
        issued.clear()
        make_terms(0)
        tick = spread(norm2_steps(jnp.minimum(i + 1, n_chunk - 1)), 7 * (n_ft - 1), x1_v, lag=6)
        act = []
        for j in range(n_ft):
            def w(r, c):
                return (wg_v, wu_v)[c][j * LANES:min((j + 1) * LANES, F), _block(r, HD)]

            if j < n_ft - 1:
                g0, u0, g1, u1 = strassen(_dot_t, 0, w, tick)
                act.append((_gelu(g0) * u0, _gelu(g1) * u1))
            else:
                g0, u0, g1, u1 = strassen(lambda h, wt: _dot_t(wt, h), 0, w, idle)
                act.append(((_gelu(g0) * u0).T.astype(BF16), (_gelu(g1) * u1).T.astype(BF16)))
        for k in range(n_pair):
            for n in range(7):
                a_terms[n, :, _block(k, LANES)] = _factor(LEFT[n], lambda half, c: act[2 * k + c][half])
        for j in range(2):
            cols = [slice((2 * j + c) * LANES, (2 * j + c + 1) * LANES) for c in range(2)]

            def w(r, c):
                return jnp.concatenate([wd_v[_block(2 * k + r, LANES), cols[c]] for k in range(n_pair)], axis=0)

            def product(n):
                return _dot(a_terms[n], _factor(RIGHT[n], w))

            def rest(half, c):
                return _dot(act[-1][half], wd_v[2 * n_pair * LANES:F, cols[c]])

            def finish(half, c, y):
                at = token_rows(i, half, 0, HM), cols[c]
                out_v[at] = (x1_v[at] + mod(5)[:, cols[c]] * y).astype(out_v.dtype)
                pltpu.make_async_copy(out_v.at[at], out_hbm.at[at], out_sem).start()

            m1, m2, m3 = product(0), product(1), product(2)
            c11, c12, c21, c22 = m1 + rest(0, 0), m3 + rest(0, 1), m2 + rest(1, 0), (m1 - m2 + m3) + rest(1, 1)
            m4 = product(3)
            finish(1, 0, c21 + m4)
            m5 = product(4)
            finish(0, 1, c12 + m5)
            finish(1, 1, c22 + product(5))
            finish(0, 0, (c11 + m4 - m5) + product(6))

    lax.fori_loop(0, n_chunk, ffn, None)
    pltpu.make_async_copy(out_v, out_hbm, out_sem).wait()


@jax.jit
def pallas_adaLN_cond__mha_block__geglu_ffn__prompt_kernel(
    A_x: jax.Array,
    A_wqkv: jax.Array,
    A_wo: jax.Array,
    B_x: jax.Array,
    B_w_gate: jax.Array,
    B_w_up: jax.Array,
    B_w_down: jax.Array,
    c: jax.Array,
    w_mod: jax.Array,
):
    del B_x
    hbm = pl.BlockSpec(memory_space=pltpu.HBM)
    vmem = pltpu.VMEM
    out = pl.pallas_call(
        _kernel,
        name="adaln_blk",
        out_shape=jax.ShapeDtypeStruct((S, D), A_x.dtype),
        in_specs=[hbm] * 8,
        out_specs=hbm,
        scratch_shapes=[
            vmem((1, D), BF16),
            vmem((S + 16, D), BF16),
            vmem((D, 3 * D), BF16),
            vmem((D, D), BF16),
            vmem((F, D), BF16),
            vmem((F, D), BF16),
            vmem((F, D), BF16),
            vmem((D, 6 * D), BF16),
            vmem((SUB, 6 * D), F32),
            _attention_scratch(),
            vmem((SUB + TM, D), F32),
            vmem((2, 7, HM, HD), F32),
            vmem((7, HD, HD), BF16),
            vmem((7, HM, F // (2 * LANES) * LANES), F32),
            vmem((S + 16, D), F32),
            vmem((S, D), BF16),
            pltpu.SemaphoreType.DMA((13,)),
            pltpu.SemaphoreType.DMA(()),
        ],
        compiler_params=pltpu.CompilerParams(vmem_limit_bytes=100 * 2**20, disable_bounds_checks=True),
    )(c, A_x.reshape(S, D), A_wqkv, A_wo, B_w_gate.T, B_w_up.T, B_w_down, w_mod)
    return out.reshape(A_x.shape)
```
